```python
import os as _os
_os.environ.setdefault("JAX_PLATFORMS", "cpu")
import jax
import jax.numpy as jnp

def _softmax(x, axis=-1):
    return jax.nn.softmax(x, axis=axis)
def _gelu(x):
    return jax.nn.gelu(x, approximate=True)
def _silu(x):
    return jax.nn.silu(x)
def _sigmoid(x):
    return jax.nn.sigmoid(x)
def _layernorm(x, axis=-1, eps=1e-5):
    m = jnp.mean(x, axis=axis, keepdims=True)
    v = jnp.var(x, axis=axis, keepdims=True)
    return (x - m) / jnp.sqrt(v + eps)
def _scatter_add(tgt, idx, src, axis=0):
    return tgt.at[idx].add(src)
def _segment_sum(src, seg, n):
    return jax.ops.segment_sum(src, seg, n)
class _Rng:
    def __init__(self, key):
        self._k = key
    def _next(self):
        self._k, sub = jax.random.split(self._k)
        return sub
    def normal(self, shape):
        return jax.random.normal(self._next(), shape, dtype=jnp.bfloat16)
    def randint(self, lo, hi, shape):
        return jax.random.randint(self._next(), shape, lo, hi, dtype=jnp.int32)
    def uniform(self, shape, lo=0.0, hi=1.0):
        return jax.random.uniform(self._next(), shape, jnp.bfloat16, lo, hi)
    def permutation(self, n):
        return jax.random.permutation(self._next(), n)


kernel_name = 'concat_heads__ssm_conv_h3__sliding_block__prompt'

def setup_inputs():
    _rng = _Rng(jax.random.key(int.from_bytes(__import__("os").urandom(4), "little")))
    _w = (lambda a: (lambda t: t.astype(jnp.bfloat16) if jnp.issubdtype(t.dtype, jnp.floating) else t)(jnp.asarray(a)))
    def _A_setup():
        B, S, D = 1, 2048, 512
        ks = 4
        return {
            "q": _w((lambda *s: _rng.normal(s) * 0.05)(B, S, D)),
            "k": _w((lambda *s: _rng.normal(s) * 0.2)(B, S, D)),
            "v": _w((lambda *s: _rng.normal(s) * 0.2)(B, S, D)),
            "shift_k": _w((lambda *s: _rng.normal(s) * 0.2)(D, ks) * 0.5),
            "ssm_k": _w((lambda *s: _rng.normal(s) * 0.2)(D, S) * (1.0 / S ** 0.5)),
            "ssm_D": _w((lambda *s: _rng.normal(s) * 0.2)(D)),
        }
    _A_in = _A_setup()

    def _B_setup():
        B, S, D = 1, 2048, 512
        return {
            "x": _w((lambda *s: _rng.normal(s) * 0.2)(B, S, D)),
            "wqkv": _w((lambda *s: _rng.normal(s) * 0.2)(D, 3 * D)),
            "wo": _w((lambda *s: _rng.normal(s) * 0.05)(D, D)),
        }
    _B_in = _B_setup()

    return {
        "A_q": _A_in["q"],
        "A_k": _A_in["k"],
        "A_v": _A_in["v"],
        "A_shift_k": _A_in["shift_k"],
        "A_ssm_k": _A_in["ssm_k"],
        "A_ssm_D": _A_in["ssm_D"],
        "B_x": _B_in["x"],
        "B_wqkv": _B_in["wqkv"],
        "B_wo": _B_in["wo"],
    }

def reference(A_q, A_k, A_v, A_shift_k, A_ssm_k, A_ssm_D, B_x, B_wqkv, B_wo):
    def _A_ref(q, k, v, shift_k, ssm_k, ssm_D):
        B, S, D = q.shape
        ks = shift_k.shape[-1]
        k_pad = jnp.pad(k, ((0, 0), (ks - 1, 0), (0, 0)))
        k_shift = jnp.zeros_like(k)
        for t in range(ks):
            k_shift = k_shift + k_pad[:, t:t + S, :] * shift_k[:, ks - 1 - t][None, None, :]
        kv = k_shift * v
        L = 2 * S
        kv_pad = jnp.pad(kv, ((0, 0), (0, S), (0, 0)))
        kf_pad = jnp.pad(ssm_k, ((0, 0), (0, S)))
        kv_f = (lambda x, axes=(-2,-1): jnp.fft.rfft2(x.astype(jnp.float32), axes=axes))(kv_pad[:, None, :, :], axes=(1, 2))
        kf_f = (lambda x, axes=(-2,-1): jnp.fft.rfft2(x.astype(jnp.float32), axes=axes))(kf_pad[:, None, :], axes=(1, 2))
        kf_f = (lambda x, *d: x.transpose(*d))(kf_f, 1, 2, 0)
        y_f = kv_f * kf_f[None, :, :, :]
        y = (lambda x, s, axes=(-2,-1): jnp.fft.irfft2(x, s=s, axes=axes).astype(jnp.bfloat16))(y_f, (1, L), axes=(1, 2))[:, 0, :S, :]
        y = y + kv * ssm_D[None, None, :]
        return q * y

    def _B_ref(x, wqkv, wo):
        B, S, D = x.shape
        H = 32; Dh = D // H; W = 256
        qkv = (lambda x, *d: x.transpose(*d))((x @ wqkv).reshape(B, S, 3, H, Dh), 2, 0, 3, 1, 4)
        q, k, v = qkv[0], qkv[1], qkv[2]
        scores = jnp.einsum("bhqd,bhkd->bhqk", q, k) * (Dh ** -0.5)
        idx = jnp.arange(S)
        mask = (idx[:, None] - idx[None, :] >= 0) & (idx[:, None] - idx[None, :] < W)
        scores = jnp.where(mask[None, None], scores, -1e9)
        p = _softmax(scores, axis=-1)
        o = jnp.einsum("bhqk,bhkd->bhqd", p, v)
        return (lambda x, *d: x.transpose(*d))(o, 0, 2, 1, 3).reshape(B, S, D) @ wo

    a = _A_ref(A_q, A_k, A_v, A_shift_k, A_ssm_k, A_ssm_D)
    b = _B_ref(B_x, B_wqkv, B_wo)
    return jnp.concatenate([a, b], axis=-1)
```

```python
import numpy as np
import jax
import jax.numpy as jnp
from jax import lax
import jax.experimental.pallas as pl
import jax.experimental.pallas.tpu as pltpu

S, D, KS = 2048, 512, 4
L = 2 * S
W = 256
BF = jnp.bfloat16
F32 = jnp.float32
NEG = -1e30


def _consts():
    n2 = np.arange(64)[:, None, None]
    k1 = np.arange(32)[None, :, None]
    n1 = np.arange(32)[None, None, :]
    th = 2 * np.pi * (64 * n1 + n2) * (k1 + 0.5) / L
    f1 = np.concatenate([np.cos(th), -np.sin(th)], axis=1)
    g = np.transpose(f1, (0, 2, 1)) * (2.0 / L)
    a = np.arange(64)
    ph = 2 * np.pi * np.outer(a, a) / 64
    c, s = np.cos(ph), -np.sin(ph)
    f2 = np.block([[c, -s], [s, c]])
    f2i = np.block([[c, s], [-s, c]])
    return (f1.astype(np.float32), g.astype(np.float32),
            np.stack([f2, f2i]).astype(np.float32))


_F1, _G, _F2 = _consts()


def _dot(a, b, dims=((1,), (0,))):
    return lax.dot_general(a, b, (dims, ((), ())), preferred_element_type=F32)


def _kernel(q_ref, k_ref, v_ref, sh_ref, kk_ref, sd_ref, x_ref, wqkv_ref, wo_ref,
            f1_ref, g_ref, f2_ref, o_ref,
            kp_ref, u_ref, a_ref, c_ref, y_ref, qs_ref, ks_ref, vt_ref, ot_ref, wvt_ref):
    kp_ref[0:8, :] = jnp.zeros((8, D), F32)
    kp_ref[8:8 + S, :] = k_ref[...].astype(F32)

    def ld(ref, n, sl):
        return jnp.concatenate([ref[j, sl, :] for j in range(n)], 1)

    def stt(ref, n, sl, val):
        for j in range(n):
            ref[j, sl, :] = val[:, j * 128:(j + 1) * 128]

    def pre(i, _):
        r = pl.multiple_of(i * 128, 128)
        blk = kp_ref[pl.ds(r, 136), :]
        acc = blk[8:] * sh_ref[0:1, :]
        for t in range(1, KS):
            acc += blk[8 - t:136 - t] * sh_ref[t:t + 1, :]
        stt(u_ref, 4, pl.ds(r, 128), acc * v_ref[pl.ds(r, 128), :].astype(F32))
        for c in range(4):
            u_ref[4 + c, pl.ds(r, 128), :] = (
                kk_ref[i, c * 128:(c + 1) * 128, :].astype(F32).T)
        return 0
    lax.fori_loop(0, 16, pre, 0)

    def st1(n2, _):
        xx = ld(u_ref, 8, pl.ds(n2, 32, stride=64)).astype(BF)
        stt(a_ref, 8, pl.ds(pl.multiple_of(n2 * 64, 64), 64), _dot(f1_ref[n2].astype(BF), xx))
        return 0
    lax.fori_loop(0, 64, st1, 0)

    def st2(k1, _):
        ar = ld(a_ref, 8, pl.ds(k1, 64, stride=64))
        ai = ld(a_ref, 8, pl.ds(k1 + 32, 64, stride=64))
        z = _dot(f2_ref[0].astype(BF), jnp.concatenate([ar, ai], 0).astype(BF))
        ur, ui, kr, ki = z[:64, :D], z[64:, :D], z[:64, D:], z[64:, D:]
        y = jnp.concatenate([ur * kr - ui * ki, ur * ki + ui * kr], 0).astype(BF)
        c = _dot(f2_ref[1].astype(BF), y)
        stt(c_ref, 4, pl.ds(k1, 64, stride=64), c[:64])
        stt(c_ref, 4, pl.ds(k1 + 32, 64, stride=64), c[64:])
        return 0
    lax.fori_loop(0, 32, st2, 0)

    def st3(n2, _):
        cc = ld(c_ref, 4, pl.ds(pl.multiple_of(n2 * 64, 64), 64)).astype(BF)
        stt(y_ref, 4, pl.ds(n2, 32, stride=64), _dot(g_ref[n2].astype(BF), cc))
        return 0
    lax.fori_loop(0, 64, st3, 0)

    def fin(i, _):
        r = pl.ds(pl.multiple_of(i * 128, 128), 128)
        y = ld(y_ref, 4, r) + ld(u_ref, 4, r) * sd_ref[...]
        o_ref[r, 0:D] = (q_ref[r, :].astype(F32) * y).astype(BF)
        return 0
    lax.fori_loop(0, 16, fin, 0)

    wvt_ref[...] = wqkv_ref[:, 2 * D:].astype(F32).T.astype(BF)
    ks_ref[:, 0:W, :] = jnp.zeros((4, W, 128), BF)
    vt_ref[0:2] = jnp.zeros((2, D, 128), BF)
    sc = 0.25 * 1.4426950408889634

    def proj(i, _):
        r = pl.multiple_of(i * 256, 256)
        xb = x_ref[pl.ds(r, 256), :]
        qq = (_dot(xb, wqkv_ref[:, 0:D]) * sc).astype(BF)
        kk = _dot(xb, wqkv_ref[:, D:2 * D]).astype(BF)
        vt = _dot(wvt_ref[...], xb, ((1,), (1,))).astype(BF)
        for g in range(4):
            qs_ref[g, pl.ds(r, 256), :] = qq[:, g * 128:(g + 1) * 128]
            ks_ref[g, pl.ds(r + W, 256), :] = kk[:, g * 128:(g + 1) * 128]
        vt_ref[2 * i + 2] = vt[:, :128]
        vt_ref[2 * i + 3] = vt[:, 128:]
        return 0
    lax.fori_loop(0, 8, proj, 0)

    lane = lax.broadcasted_iota(jnp.int32, (64, 128), 1)
    row = lax.broadcasted_iota(jnp.int32, (64, 128), 0)
    m_lo = row > (lane % 64)
    lane16 = lax.broadcasted_iota(jnp.int32, (64, 128), 1) // 16
    half = lax.broadcasted_iota(jnp.int32, (16, 128), 1) < 64

    def attn(i, first):
        r = i * 128 if first else pl.multiple_of(i * 128, 128)
        for g in range(4):
            for p in range(4):
                outs = []
                for t in range(2):
                    qb = qs_ref[g, pl.ds(r + 64 * t, 64), :]
                    z = jnp.zeros_like(qb)
                    qm = jnp.concatenate([jnp.where(lane16 == 2 * p, qb, z),
                                          jnp.where(lane16 == 2 * p + 1, qb, z)], 0)
                    kb = ks_ref[g, pl.ds(r + 64 * t, 320), :]
                    s = _dot(kb, qm, ((1,), (1,)))
                    s0 = jnp.where(m_lo, s[:64], NEG)
                    s2 = jnp.where(m_lo, NEG, s[256:])
                    s1 = s[64:256]
                    if first:
                        lo = W - (128 * i + 64 * t)
                        s0 = jnp.where(row >= lo, s0, NEG)
                        rr = lax.broadcasted_iota(jnp.int32, (192, 128), 0) + 64
                        s1 = jnp.where(rr >= lo, s1, NEG)
                    m = jnp.maximum(jnp.maximum(s0, s2),
                                    jnp.maximum(jnp.maximum(s1[:64], s1[64:128]), s1[128:]))
                    m = jnp.max(m, axis=0, keepdims=True)
                    e0, e1, e2 = jnp.exp2(s0 - m), jnp.exp2(s1 - m), jnp.exp2(s2 - m)
                    l = jnp.sum(e0 + e2 + e1[:64] + e1[64:128] + e1[128:], axis=0, keepdims=True)
                    zz = jnp.zeros((64, 128), BF)
                    pp = [e0.astype(BF), e1.astype(BF), e2.astype(BF)]
                    pp = pp + [zz] if t == 0 else [zz] + pp
                    pt = jnp.concatenate(pp, 0)
                    rs = pl.ds(g * 128 + p * 32, 32)
                    vt = jnp.concatenate([vt_ref[i, rs, :], vt_ref[i + 1, rs, :],
                                          vt_ref[i + 2, rs, :]], 1)
                    outs.append(_dot(vt, pt) * (1.0 / l))
                o1, o2 = outs
                o2r = pltpu.roll(o2, 64, 1)
                o1r = pltpu.roll(o1, 64, 1)
                oa = jnp.where(half, o1[:16], o2r[:16])
                ob = jnp.where(half, o1r[16:], o2[16:])
                ot_ref[i, pl.ds(g * 128 + p * 32, 32), :] = jnp.concatenate([oa, ob], 0).astype(BF)

    attn(0, True)
    attn(1, True)

    def ab(i, _):
        attn(i, False)
        return 0
    lax.fori_loop(2, 16, ab, 0)

    def ob_(i, _):
        r = pl.ds(pl.multiple_of(i * 128, 128), 128)
        o_ref[r, D:2 * D] = _dot(ot_ref[i], wo_ref[...], ((0,), (0,))).astype(BF)
        return 0
    lax.fori_loop(0, 16, ob_, 0)


@jax.jit
def pallas_concat_heads__ssm_conv_h3__sliding_block__prompt_kernel(
    A_q, A_k, A_v, A_shift_k, A_ssm_k, A_ssm_D, B_x, B_wqkv, B_wo):
    sh = A_shift_k.T.astype(F32)
    kk = A_ssm_k.reshape(D, 16, 128).transpose(1, 0, 2)
    out = pl.pallas_call(
        _kernel,
        out_shape=jax.ShapeDtypeStruct((S, 2 * D), BF),
        scratch_shapes=[
            pltpu.VMEM((S + 8, D), F32),
            pltpu.VMEM((8, S, 128), F32),
            pltpu.VMEM((8, L, 128), F32),
            pltpu.VMEM((4, L, 128), F32),
            pltpu.VMEM((4, S, 128), F32),
            pltpu.VMEM((4, S, 128), BF),
            pltpu.VMEM((4, S + W, 128), BF),
            pltpu.VMEM((18, D, 128), BF),
            pltpu.VMEM((16, D, 128), BF),
            pltpu.VMEM((D, D), BF),
        ],
        compiler_params=pltpu.CompilerParams(vmem_limit_bytes=120 * 1024 * 1024),
    )(A_q[0], A_k[0], A_v[0], sh, kk, A_ssm_D.astype(F32).reshape(1, D),
      B_x[0], B_wqkv, B_wo, _F1, _G, _F2)
    return out[None]
```

```python
import numpy as np
import jax
import jax.numpy as jnp
from jax import lax
import jax.experimental.pallas as pl
import jax.experimental.pallas.tpu as pltpu

S, D, KS = 2048, 512, 4
L = 2 * S
W = 256
BF = jnp.bfloat16
F32 = jnp.float32
NEG = -1e30
P = 68


def _consts():
    n2 = np.arange(64)[:, None, None]
    k1 = np.arange(32)[None, :, None]
    n1 = np.arange(32)[None, None, :]
    th = 2 * np.pi * (64 * n1 + n2) * (k1 + 0.5) / L
    f1 = np.concatenate([np.cos(th), -np.sin(th)], axis=1)
    g = np.transpose(f1, (0, 2, 1)) * (2.0 / L)
    a = np.arange(64)
    ph = 2 * np.pi * np.outer(a, a) / 64
    c, s = np.cos(ph), -np.sin(ph)
    f2 = np.block([[c, -s], [s, c]])
    f2i = np.block([[c, s], [-s, c]])
    return (f1.astype(jnp.bfloat16), g.astype(jnp.bfloat16),
            np.stack([f2, f2i]).astype(jnp.bfloat16))


_F1, _G, _F2 = _consts()


def _dot(a, b, dims=((1,), (0,))):
    return lax.dot_general(a, b, (dims, ((), ())), preferred_element_type=F32)


def _kernel(q_h, k_h, v_h, kk_h, x_h, wqkv_h, wo_h, sh16, sd16,
            f1_ref, g_ref, f2_ref, o_h,
            q_ref, k_ref, v_ref, kk_ref, x_ref, wqkv_ref, wo_ref, o_ref, sem,
            kp_ref, u_ref, a_ref, c_ref, y_ref, qs_ref, ks_ref, vt_ref, ot_ref, wvt_ref):
    cps = [pltpu.make_async_copy(a, b, sem.at[j]) for j, (a, b) in enumerate(
        [(k_h, k_ref), (v_h, v_ref), (kk_h, kk_ref), (q_h, q_ref),
         (wqkv_h, wqkv_ref), (x_h, x_ref), (wo_h, wo_ref)])]
    for c in cps[:3]:
        c.start()
    shv = sh16[...].astype(F32)
    sdv = sd16[...].astype(F32)
    cps[0].wait()
    kp_ref[0:8, :] = jnp.zeros((8, D), F32)
    kp_ref[8:8 + S, :] = k_ref[...].astype(F32)

    cps[1].wait()
    cps[2].wait()
    for c in cps[3:]:
        c.start()

    def ld(ref, n, sl):
        return jnp.concatenate([ref[j, sl, :] for j in range(n)], 1)

    def stt(ref, n, sl, val):
        for j in range(n):
            ref[j, sl, :] = val[:, j * 128:(j + 1) * 128]

    def pre(i, _):
        r = pl.multiple_of(i * 128, 128)
        blk = kp_ref[pl.ds(r, 136), :]
        acc = blk[8:] * shv[0:1]
        for t in range(1, KS):
            acc += blk[8 - t:136 - t] * shv[t:t + 1]
        kv = acc * v_ref[pl.ds(r, 128), :].astype(F32)
        for h in range(2):
            rr = pl.ds((2 * i + h) * P, 64, stride=1)
            stt(u_ref, 4, rr, kv[h * 64:(h + 1) * 64])
            for c in range(4):
                u_ref[4 + c, rr, :] = (
                    kk_ref[c * 128:(c + 1) * 128, pl.ds(r, 128)].astype(F32).T)[h * 64:(h + 1) * 64]
        return 0
    with jax.named_scope('pre'):
        lax.fori_loop(0, 16, pre, 0)

    def st1(n2, _):
        xx = ld(u_ref, 8, pl.ds(n2, 32, stride=P)).astype(BF)
        stt(a_ref, 8, pl.ds(n2 * P, 64, stride=1), _dot(f1_ref[n2].astype(BF), xx))
        return 0
    with jax.named_scope('st1'):
        lax.fori_loop(0, 64, st1, 0, unroll=8)

    def st2(k1, _):
        ar = ld(a_ref, 8, pl.ds(k1, 64, stride=P))
        ai = ld(a_ref, 8, pl.ds(k1 + 32, 64, stride=P))
        z = _dot(f2_ref[0].astype(BF), jnp.concatenate([ar, ai], 0).astype(BF))
        ur, ui, kr, ki = z[:64, :D], z[64:, :D], z[:64, D:], z[64:, D:]
        y = jnp.concatenate([ur * kr - ui * ki, ur * ki + ui * kr], 0).astype(BF)
        c = _dot(f2_ref[1].astype(BF), y)
        stt(c_ref, 4, pl.ds(k1, 64, stride=P), c[:64])
        stt(c_ref, 4, pl.ds(k1 + 32, 64, stride=P), c[64:])
        return 0
    with jax.named_scope('st2'):
        lax.fori_loop(0, 32, st2, 0, unroll=4)

    def st3(n2, _):
        cc = ld(c_ref, 4, pl.ds(n2 * P, 64, stride=1)).astype(BF)
        stt(y_ref, 4, pl.ds(n2, 32, stride=P), _dot(g_ref[n2].astype(BF), cc))
        return 0
    with jax.named_scope('st3'):
        lax.fori_loop(0, 64, st3, 0, unroll=4)

    cps[3].wait()

    def fin(i, _):
        r = pl.ds(pl.multiple_of(i * 64, 64), 64)
        rr = pl.ds(i * P, 64, stride=1)
        y = ld(y_ref, 4, rr) + ld(u_ref, 4, rr) * sdv
        o_ref[r, 0:D] = (q_ref[r, :].astype(F32) * y).astype(BF)
        return 0
    with jax.named_scope('fin'):
        lax.fori_loop(0, 32, fin, 0)

    oa = pltpu.make_async_copy(o_ref.at[:, 0:D], o_h.at[:, 0:D], sem.at[7])
    oa.start()
    cps[4].wait()
    cps[5].wait()
    wvt_ref[...] = wqkv_ref[:, 2 * D:].astype(F32).T.astype(BF)
    ks_ref[:, 0:W, :] = jnp.zeros((4, W, 128), BF)
    vt_ref[0:2] = jnp.zeros((2, D, 128), BF)
    sc = 0.25 * 1.4426950408889634

    def proj(i, _):
        r = pl.multiple_of(i * 256, 256)
        xb = x_ref[pl.ds(r, 256), :]
        qq = (_dot(xb, wqkv_ref[:, 0:D]) * sc).astype(BF)
        kk = _dot(xb, wqkv_ref[:, D:2 * D]).astype(BF)
        vt = _dot(wvt_ref[...], xb, ((1,), (1,))).astype(BF)
        for g in range(4):
            qs_ref[g, pl.ds(r, 256), :] = qq[:, g * 128:(g + 1) * 128]
            ks_ref[g, pl.ds(r + W, 256), :] = kk[:, g * 128:(g + 1) * 128]
        vt_ref[2 * i + 2] = vt[:, :128]
        vt_ref[2 * i + 3] = vt[:, 128:]
        return 0
    with jax.named_scope('proj'):
        lax.fori_loop(0, 8, proj, 0)

    lane = lax.broadcasted_iota(jnp.int32, (64, 128), 1)
    row = lax.broadcasted_iota(jnp.int32, (64, 128), 0)
    m_lo = row > (lane % 64)
    lane16 = lax.broadcasted_iota(jnp.int32, (64, 128), 1) // 16
    l16 = lax.broadcasted_iota(jnp.int32, (32, 128), 1) // 16
    hm = [jnp.where(l16 == h, jnp.uint32(0xFFFFFFFF), jnp.uint32(0)) for h in range(8)]
    half = lax.broadcasted_iota(jnp.int32, (16, 128), 1) < 64

    def attn(i, first):
        r = i * 128 if first else pl.multiple_of(i * 128, 128)
        def qk(g):
            sall = []
            for t in range(2):
                qb = pltpu.bitcast(qs_ref[g, pl.ds(r + 64 * t, 64), :], jnp.uint32)
                qm = pltpu.bitcast(jnp.concatenate([qb & hm[h] for h in range(8)], 0), BF)
                kb = ks_ref[g, pl.ds(r + 64 * t, 320), :]
                sall.append(_dot(kb, qm, ((1,), (1,))))
            return sall
        nxt = qk(0)
        for g in range(4):
            sall = nxt
            if g < 3:
                nxt = qk(g + 1)
            for p in range(4):
                outs = []
                for t in range(2):
                    s = sall[t][:, p * 128:(p + 1) * 128]
                    s0 = jnp.where(m_lo, s[:64], NEG)
                    s2 = jnp.where(m_lo, NEG, s[256:])
                    s1 = s[64:256]
                    if first:
                        lo = W - (128 * i + 64 * t)
                        s0 = jnp.where(row >= lo, s0, NEG)
                        rr = lax.broadcasted_iota(jnp.int32, (192, 128), 0) + 64
                        s1 = jnp.where(rr >= lo, s1, NEG)
                    m = jnp.maximum(jnp.maximum(s0, s2),
                                    jnp.maximum(jnp.maximum(s1[:64], s1[64:128]), s1[128:]))
                    m = jnp.max(m, axis=0, keepdims=True)
                    e0, e1, e2 = jnp.exp2(s0 - m), jnp.exp2(s1 - m), jnp.exp2(s2 - m)
                    l = jnp.sum(e0 + e2 + e1[:64] + e1[64:128] + e1[128:], axis=0, keepdims=True)
                    zz = jnp.zeros((64, 128), BF)
                    pp = [e0.astype(BF), e1.astype(BF), e2.astype(BF)]
                    pp = pp + [zz] if t == 0 else [zz] + pp
                    pt = jnp.concatenate(pp, 0)
                    rs = pl.ds(g * 128 + p * 32, 32)
                    vt = jnp.concatenate([vt_ref[i, rs, :], vt_ref[i + 1, rs, :],
                                          vt_ref[i + 2, rs, :]], 1)
                    outs.append(_dot(vt, pt) * (1.0 / l))
                o1, o2 = outs
                o2r = pltpu.roll(o2, 64, 1)
                o1r = pltpu.roll(o1, 64, 1)
                o_a = jnp.where(half, o1[:16], o2r[:16])
                ob = jnp.where(half, o1r[16:], o2[16:])
                ot_ref[i, pl.ds(g * 128 + p * 32, 32), :] = jnp.concatenate([o_a, ob], 0).astype(BF)

    with jax.named_scope('a01'):
        attn(0, True)
        attn(1, True)

    def ab(i, _):
        attn(i, False)
        return 0
    with jax.named_scope('ab'):
        lax.fori_loop(2, 16, ab, 0)

    cps[6].wait()

    def ocp(j):
        r = pl.ds(pl.multiple_of(j * 512, 512), 512)
        return pltpu.make_async_copy(o_ref.at[r, D:], o_h.at[r, D:], sem.at[8 + j])

    def ob_(j, _):
        for h in range(4):
            i = j * 4 + h
            r = pl.ds(pl.multiple_of(i * 128, 128), 128)
            o_ref[r, D:2 * D] = _dot(ot_ref[i], wo_ref[...], ((0,), (0,))).astype(BF)
        ocp(j).start()
        return 0
    with jax.named_scope('ob_'):
        lax.fori_loop(0, 4, ob_, 0)
    for j in range(4):
        ocp(j).wait()
    oa.wait()


@jax.jit
def pallas_concat_heads__ssm_conv_h3__sliding_block__prompt_kernel(
    A_q, A_k, A_v, A_shift_k, A_ssm_k, A_ssm_D, B_x, B_wqkv, B_wo):
    anys = pl.BlockSpec(memory_space=pl.ANY)
    out = pl.pallas_call(
        _kernel,
        out_shape=jax.ShapeDtypeStruct((S, 2 * D), BF),
        in_specs=[anys] * 7 + [pl.BlockSpec(memory_space=pltpu.VMEM)] * 5,
        out_specs=anys,
        scratch_shapes=[
            pltpu.VMEM((S, D), BF), pltpu.VMEM((S, D), BF), pltpu.VMEM((S, D), BF),
            pltpu.VMEM((D, S), BF), pltpu.VMEM((S, D), BF), pltpu.VMEM((D, 3 * D), BF),
            pltpu.VMEM((D, D), BF), pltpu.VMEM((S, 2 * D), BF),
            pltpu.SemaphoreType.DMA((12,)),
            pltpu.VMEM((S + 8, D), F32),
            pltpu.VMEM((8, 32 * P, 128), F32),
            pltpu.VMEM((8, 64 * P, 128), F32),
            pltpu.VMEM((4, 64 * P, 128), F32),
            pltpu.VMEM((4, 32 * P, 128), F32),
            pltpu.VMEM((4, S, 128), BF),
            pltpu.VMEM((4, S + W, 128), BF),
            pltpu.VMEM((18, D, 128), BF),
            pltpu.VMEM((16, D, 128), BF),
            pltpu.VMEM((D, D), BF),
        ],
        compiler_params=pltpu.CompilerParams(vmem_limit_bytes=120 * 1024 * 1024),
    )(A_q[0], A_k[0], A_v[0], A_ssm_k, B_x[0], B_wqkv, B_wo,
      A_shift_k.T, A_ssm_D.reshape(1, D), _F1, _G, _F2)
    return out[None]
```
